```python
import os as _os
_os.environ.setdefault("JAX_PLATFORMS", "cpu")
import jax
import jax.numpy as jnp

def _softmax(x, axis=-1):
    return jax.nn.softmax(x, axis=axis)
def _gelu(x):
    return jax.nn.gelu(x, approximate=True)
def _silu(x):
    return jax.nn.silu(x)
def _sigmoid(x):
    return jax.nn.sigmoid(x)
def _layernorm(x, axis=-1, eps=1e-5):
    m = jnp.mean(x, axis=axis, keepdims=True)
    v = jnp.var(x, axis=axis, keepdims=True)
    return (x - m) / jnp.sqrt(v + eps)
def _scatter_add(tgt, idx, src, axis=0):
    return tgt.at[idx].add(src)
def _segment_sum(src, seg, n):
    return jax.ops.segment_sum(src, seg, n)
class _Rng:
    def __init__(self, key):
        self._k = key
    def _next(self):
        self._k, sub = jax.random.split(self._k)
        return sub
    def normal(self, shape):
        return jax.random.normal(self._next(), shape, dtype=jnp.bfloat16)
    def randint(self, lo, hi, shape):
        return jax.random.randint(self._next(), shape, lo, hi, dtype=jnp.int32)
    def uniform(self, shape, lo=0.0, hi=1.0):
        return jax.random.uniform(self._next(), shape, jnp.bfloat16, lo, hi)
    def permutation(self, n):
        return jax.random.permutation(self._next(), n)


kernel_name = 'concat_heads__mha_block_cached__mha_block_cached__near_ridge'

def setup_inputs():
    _rng = _Rng(jax.random.key(int.from_bytes(__import__("os").urandom(4), "little")))
    _w = (lambda a: (lambda t: t.astype(jnp.bfloat16) if jnp.issubdtype(t.dtype, jnp.floating) else t)(jnp.asarray(a)))
    def _A_setup():
        B, Sq, D = 16, 80, 512
        H, Sk, Dh = 32, 80, 128
        return {
            "x": _w((lambda *s: _rng.normal(s) * 0.8)(B, Sq, D)),
            "k_cache": _w((lambda *s: _rng.normal(s) * 0.8)(B, H, Sk, Dh)),
            "v_cache": _w((lambda *s: _rng.normal(s) * 0.05)(B, H, Sk, Dh)),
            "wq": _w((lambda *s: _rng.normal(s) * 0.8)(D, H * Dh) * (D ** -0.5)),
            "wo": _w((lambda *s: _rng.normal(s) * 0.05)(H * Dh, D) * ((H * Dh) ** -0.5)),
        }
    _A_in = _A_setup()

    def _B_setup():
        B, Sq, D = 16, 80, 512
        H, Sk, Dh = 32, 80, 128
        return {
            "x": _w((lambda *s: _rng.normal(s) * 0.8)(B, Sq, D)),
            "k_cache": _w((lambda *s: _rng.normal(s) * 0.8)(B, H, Sk, Dh)),
            "v_cache": _w((lambda *s: _rng.normal(s) * 0.05)(B, H, Sk, Dh)),
            "wq": _w((lambda *s: _rng.normal(s) * 0.8)(D, H * Dh) * (D ** -0.5)),
            "wo": _w((lambda *s: _rng.normal(s) * 0.05)(H * Dh, D) * ((H * Dh) ** -0.5)),
        }
    _B_in = _B_setup()

    return {
        "A_x": _A_in["x"],
        "A_k_cache": _A_in["k_cache"],
        "A_v_cache": _A_in["v_cache"],
        "A_wq": _A_in["wq"],
        "A_wo": _A_in["wo"],
        "B_x": _B_in["x"],
        "B_k_cache": _B_in["k_cache"],
        "B_v_cache": _B_in["v_cache"],
        "B_wq": _B_in["wq"],
        "B_wo": _B_in["wo"],
    }

def reference(A_x, A_k_cache, A_v_cache, A_wq, A_wo, B_x, B_k_cache, B_v_cache, B_wq, B_wo):
    def _A_ref(x, k_cache, v_cache, wq, wo):
        B, Sq, D = x.shape
        H, Dh = 32, 128
        q = (lambda x, *d: x.transpose(*d))((x @ wq).reshape(B, Sq, H, Dh), 0, 2, 1, 3)
        scores = jnp.einsum("bhqd,bhkd->bhqk", q, k_cache) * (Dh ** -0.5)
        p = _softmax(scores, axis=-1)
        o = jnp.einsum("bhqk,bhkd->bhqd", p, v_cache)
        return (lambda x, *d: x.transpose(*d))(o, 0, 2, 1, 3).reshape(B, Sq, H * Dh) @ wo

    def _B_ref(x, k_cache, v_cache, wq, wo):
        B, Sq, D = x.shape
        H, Dh = 32, 128
        q = (lambda x, *d: x.transpose(*d))((x @ wq).reshape(B, Sq, H, Dh), 0, 2, 1, 3)
        scores = jnp.einsum("bhqd,bhkd->bhqk", q, k_cache) * (Dh ** -0.5)
        p = _softmax(scores, axis=-1)
        o = jnp.einsum("bhqk,bhkd->bhqd", p, v_cache)
        return (lambda x, *d: x.transpose(*d))(o, 0, 2, 1, 3).reshape(B, Sq, H * Dh) @ wo

    a = _A_ref(A_x, A_k_cache, A_v_cache, A_wq, A_wo)
    b = _B_ref(B_x, B_k_cache, B_v_cache, B_wq, B_wo)
    return jnp.concatenate([a, b], axis=-1)
```

```python
import jax
import jax.numpy as jnp
import numpy as np
import jax.experimental.pallas as pl
import jax.experimental.pallas.tpu as pltpu

G = 4
NC = 4
NBUF = 4
LP = 1
LAGQ = 3
S = 0
CUTS = (2, 3, 5)
ECUTS = (4, 5)
O2 = (1, 2, 3, 4)
Q2 = (1, 2, 3, 4)
SPLIT = 1
EXTRA = 0
PAD = 1
LOOPONLY = 0
PRE = 2
PQ, PK, PP, PO = (0.0, 0.7), (0.0, 0.7), (0.0, 0.95), (0.3, 0.7)
PX, PF = (2.0, 1.0), (3.0, 0.7)
CW = 0.7
NORMP = 1
KV32 = 1
FLAGS = {}
B, SQ, D, H, SK, DH = 16, 80, 512, 32, 80, 128
M = B * SQ
SCALE_LOG2E = float(DH ** -0.5 * np.log2(np.e))
F32, BF16, U32 = jnp.float32, jnp.bfloat16, jnp.uint32


def _f32(a):
    return a.astype(F32)


LHS = (((0, 0), (1, 1), 1), ((1, 0), (1, 1), 1), ((0, 0),), ((1, 1),), ((0, 0), (0, 1), 1), ((1, 0), (0, 0), -1), ((0, 1), (1, 1), -1))
RHS = (((0, 0), (1, 1), 1), ((0, 0),), ((0, 1), (1, 1), -1), ((1, 0), (0, 0), -1), ((1, 1),), ((0, 0), (0, 1), 1), ((1, 0), (1, 1), 1))


def term(spec, block):
    if len(spec) == 1:
        return block(*spec[0])
    a, b = _f32(block(*spec[0])), _f32(block(*spec[1]))
    return a + b if spec[2] > 0 else a - b


def terms(side, r, split, block):
    if not split:
        return [term(side[r], block)]
    quarter = [[term(side[r], lambda i, j: block(2 * i + a, 2 * j + b)) for b in range(2)] for a in range(2)]
    return [term(spec, lambda i, j: quarter[i][j]) for spec in side]


def strassen(product, emit):
    m2 = yield from product(1)
    m4 = yield from product(3)
    emit(1, 0, m2 + m4)
    m1 = yield from product(0)
    c11, c22 = m1 + m4, m1 - m2
    m5 = yield from product(4)
    c11 = c11 - m5
    m3 = yield from product(2)
    emit(0, 1, m3 + m5)
    c22 = c22 + m3
    m7 = yield from product(6)
    emit(0, 0, c11 + m7)
    m6 = yield from product(5)
    emit(1, 1, c22 + m6)


def _cat(parts, axis):
    return parts[0] if len(parts) == 1 else jnp.concatenate(parts, axis=axis)


def interleave(gens):
    at = [[(i + 0.5) / n for i in range(n)] if isinstance(n, int) else n for _, n, _, _ in gens]
    order = sorted((g[2] + g[3] * x, k) for k, g in enumerate(gens) for x in at[k])
    left = [len(a) for a in at]
    for _, k in order:
        next(gens[k][0])
        left[k] -= 1
        if left[k] == 0:
            for _ in gens[k][0]:
                pass


def _kernel(ax, ak, av, awq, awo, bx, bk, bv, bwq, bwo, out,
            xbuf, xs, kbuf, vbuf, wqbuf, wobuf, wqs, wos, qs, es, rs, os_, acc, obuf, sem_x, sem_in, sem_out):
    nstep = H // G
    T = 2 * nstep
    CB = B // NC
    CR = CB * SQ
    R = CR // 2
    RQ = RO = R
    qbase = [sum(7 if k in Q2 else 4 for k in range(r)) for r in range(8)]
    obase = [sum(7 if k in O2 else 4 for k in range(r)) for r in range(8)]
    NQB = 1 if LAGQ < NC else 2
    WQ, KK, VV, WO = range(4)
    refs = ((awq, ak, av, awo), (bwq, bk, bv, bwo))

    def ld(ref, idx, r0=None, n=None):
        if not KV32:
            return ref[idx] if r0 is None else ref[(*idx, slice(r0, r0 + n))]
        v = ref.bitcast(U32)
        return pltpu.bitcast(v[idx] if r0 is None else v[(*idx, slice(r0 // 2, (r0 + n) // 2))], BF16)

    def dma(kind, half, br, g, slot):
        src = refs[br][kind]
        h0 = g * G
        c0 = h0 * DH if isinstance(h0, int) else pl.multiple_of(h0 * DH, DH)
        sem = sem_in.at[kind, half, slot]
        if kind == WQ:
            return pltpu.make_async_copy(src.at[:, pl.ds(c0, G * DH)], wqbuf.at[slot], sem)
        if kind == WO:
            return pltpu.make_async_copy(src.at[pl.ds(c0, G * DH), :], wobuf.at[slot], sem)
        bs = pl.ds(half * (B // SPLIT), B // SPLIT)
        return pltpu.make_async_copy(src.at[bs, pl.ds(h0, G)], (kbuf, vbuf)[kind - KK].at[slot, bs], sem)

    def rows(start, size):
        return pl.ds(start if isinstance(start, int) else pl.multiple_of(start, 16 if size % 16 == 0 else 8), size)

    QUAD = [(a, b) for a in range(2) for b in range(2)]

    def prep_x(src, dst, c, off, n):
        for p in range(0, n, 16):
            def block(i, j):
                return xbuf[src, rows(c * CR + i * SQ + off + p, 16), j * 128:(j + 1) * 128]
            for r in range(7):
                if r in Q2:
                    vals = terms(LHS, r, True, block)
                else:
                    vals = [terms(LHS, r, False, lambda i, j: block(2 * i + a, 2 * j + b))[0] for a, b in QUAD]
                for k, m in enumerate(vals):
                    xs[dst, qbase[r] + k, rows(c * SQ + off + p, 16), :] = m.astype(BF16)
            yield

    def prep_w(src, dst, base, two, t, r):
        slot = t & (NBUF - 1)
        for p in range(0, 128, 64):
            def block(i, j):
                return src[slot, i * 128 + p:i * 128 + p + 64, j * 128:(j + 1) * 128]
            if r in two:
                vals = terms(RHS, r, True, block)
            else:
                vals = [terms(RHS, r, False, lambda i, j: block(2 * i + a, 2 * j + b))[0] for a, b in QUAD]
            for k, m in enumerate(vals):
                dst[base[r] + k, p:p + 64, :] = m.astype(BF16)

    def prep_wq(t, r):
        prep_w(wqbuf, wqs, qbase, Q2, t, r)

    def prep_wo(t, r):
        prep_w(wobuf, wos, obase, O2, t, r)

    def block_dot(lhs, rhs, base, two, r, emit):
        if r in two:
            def product(k):
                m = jnp.dot(lhs(base[r] + k), ld(rhs, (base[r] + k,)), preferred_element_type=F32)
                yield
                return m
            yield from strassen(product, emit)
        else:
            a = _cat([_cat([lhs(base[r] + 2 * i + j) for j in range(2)], 1) for i in range(2)], 0)
            w = _cat([_cat([ld(rhs, (base[r] + 2 * i + j,)) for j in range(2)], 1) for i in range(2)], 0)
            m = jnp.dot(a, w, preferred_element_type=F32)
            for _ in range(7):
                yield
            for i, j in QUAD:
                emit(i, j, m[i * SQ:(i + 1) * SQ, j * 128:(j + 1) * 128])

    def qproj(t, c):
        br = t // nstep

        def product(r):
            m = {}
            yield from block_dot(lambda k: ld(xs, (br, k), c * SQ, SQ), wqs, qbase, Q2, r,
                                 lambda i, j, v: m.__setitem__((i, j), v))
            if c == NC - 1 and not (isinstance(t, int) and t + 1 >= T):
                prep_wq(t + 1, r)
            return _cat([_cat([m[i, j] for j in range(2)], 1) for i in range(2)], 0)

        def emit(i, l, v):
            for h in range(2):
                r0 = c * CR + i * R
                qs[(t & 1 if NQB > 1 else 0), l * 2 + h, r0:r0 + R, :] = v[:, h * DH:(h + 1) * DH].astype(BF16)
        yield from strassen(product, emit)

    def pairs(c):
        if O2:
            return [[(c * CB + i, j) for i in range(4) for j in range(4)]]
        return [[(c * CB + 2 * i + a, 2 * j + b) for i in range(2) for j in range(2)] for a, b in QUAD]

    def pad_keys(a):
        return jnp.concatenate([a, jnp.zeros((DH - SK, DH), BF16)], axis=0) if PAD else a

    def qk(t, c):
        slot = t & (NBUF - 1)
        for b, h in [p for grp in pairs(c) for p in grp]:
            q = ld(qs, ((t & 1 if NQB > 1 else 0), h), b * SQ, SQ)
            k = pad_keys(ld(kbuf, (slot, b, h)))
            s = jax.lax.dot_general(q, k, (((1,), (1,)), ((), ())), preferred_element_type=F32)
            if PAD:
                s = jnp.where(jax.lax.broadcasted_iota(jnp.int32, s.shape, 1) < SK, s, -jnp.inf)
            m = jnp.max(s, axis=-1, keepdims=True)
            e = jnp.exp2((s - m) * SCALE_LOG2E)
            rl = pl.reciprocal(jnp.sum(e, axis=-1, keepdims=True), approx=True)
            if NORMP:
                es[h, b * SQ:(b + 1) * SQ, :] = (e * rl).astype(BF16)
            else:
                es[h, b * SQ:(b + 1) * SQ, :] = e.astype(BF16)
                rs[h, b * SQ:(b + 1) * SQ, :] = jnp.broadcast_to(rl, (SQ, DH))
            yield

    def pv(t, c):
        slot = t & (NBUF - 1)
        for g, grp in enumerate(pairs(c)):
            o = {}
            for b, h in grp:
                o[b - c * CB, h] = jnp.dot(ld(es, (h,), b * SQ, SQ), pad_keys(ld(vbuf, (slot, b, h))), preferred_element_type=F32)
                if not NORMP:
                    o[b - c * CB, h] = o[b - c * CB, h] * rs[h, b * SQ:(b + 1) * SQ, :]
                yield
            for p in range(0, SQ, 16):
                def block(i, j):
                    return o[i, j][p:p + 16]
                for r in range(7):
                    if r in O2:
                        vals = enumerate(terms(LHS, r, True, block))
                    else:
                        vals = [(k, terms(LHS, r, False, lambda i, j: block(2 * i + a, 2 * j + b))[0])
                                for k, (a, b) in enumerate(QUAD) if O2 or k == g]
                    for k, m in vals:
                        os_[obase[r] + k, c * SQ + p:c * SQ + p + 16, :] = m.astype(BF16)
                    if O2:
                        yield

    def oproj(t, c):
        static = isinstance(t, int)
        br, first = t // nstep, (t & (nstep - 1)) == 0
        for r in range(7):
            def emit(i, j, m):
                at = (br, r, slice(c * R + i * SQ, c * R + (i + 1) * SQ), slice(j * 128, (j + 1) * 128))
                if not (static and first):
                    m = (acc[at] if static else jnp.where(first, 0.0, acc[at])) + m
                acc[at] = m
            yield from block_dot(lambda k: ld(os_, (k,), c * SQ, SQ), wos, obase, O2, r, emit)
            if c == NC - 1 and not (static and t + 1 >= T):
                prep_wo(t + 1, r)

    def out_copy(br, c):
        return pltpu.make_async_copy(obuf.at[br, pl.ds(c * CR, CR)], out.at[pl.ds(c * CR, CR), pl.ds(br * D, D)],
                                     sem_out.at[br, c])

    def finalize(src, dst, c, off, n):
        for p in range(0, n, 16):
            for a in range(0, D // 2, 128):
                def product(r):
                    return acc[src, r, rows(c * R + off + p, 16), a:a + 128]
                    yield

                def emit(i, l, v):
                    obuf[dst, rows(c * CR + i * R + off + p, 16), l * D // 2 + a:l * D // 2 + a + 128] = v.astype(BF16)
                for _ in strassen(product, emit):
                    pass
            yield

    def x_copy(br, c):
        return pltpu.make_async_copy((ax, bx)[br].at[pl.ds(c * CR, CR)], xbuf.at[br, pl.ds(c * CR, CR)], sem_x.at[br, c])

    p_steps = CB * G
    if O2:
        p_steps = [(1 - CW) * (i + 0.5) / 16 for i in range(16)] + [1 - CW + CW * (i + 0.5) / 35 for i in range(35)]
    lag = {"q": LAGQ, "k": 0, "p": -LP, "o": -LP - 1}
    fns = {"q": (qproj, 49), "k": (qk, CB * G), "p": (pv, p_steps), "o": (oproj, 49)}

    place = {"q": PQ, "k": PK, "p": PP, "o": PO}

    def stage(s, t, c, at=0):
        return (fns[s][0](t, c), fns[s][1], at + place[s][0], place[s][1])

    def unit(t, c, at=0):
        items = [(s, t + (c + lag[s]) // NC, (c + lag[s]) % NC) for s in "qkpo"]
        return [stage(*it, at) for it in items if not isinstance(t, int) or 0 <= it[1] < T]

    ahead = (S + NC - 1 + LAGQ) // NC
    x_end = nstep - ahead
    npc = nstep // 2

    def bg_x(t):
        piece = (t & (NC - 1), 0, SQ)
        return (prep_x(jnp.where(t >= x_end - npc, 1, 0), jnp.where(t < x_end, 1, 2), *piece), piece[2] // 16, *PX)

    def bg_out(t):
        piece = (t & (NC - 1), 0, R)
        return (finalize(0, jnp.where(jnp.logical_and(t >= nstep, t < nstep + npc), 0, 2), *piece), piece[2] // 16, *PF)

    x_all = pltpu.make_async_copy(bx, xbuf.at[1], sem_x.at[1, 0])
    out_a = pltpu.make_async_copy(obuf.at[0], out.at[:, pl.ds(0, D)], sem_out.at[0, 0])

    def needs(u):
        res = [("x", 0, u + LAGQ + 1)] if u + LAGQ + 1 < NC else []
        for kind, s, step in ((WQ, "q", NC), (KK, "k", NC // SPLIT), (VV, "p", NC // SPLIT), (WO, "o", NC)):
            tt, cc = divmod(u + lag[s] + (s in "qo"), NC)
            if cc % step == 0 and 0 <= tt < T and (tt > 0 or kind != WQ):
                res.append((kind, cc // step, tt))
        return res

    def copy_of(need):
        kind, half, tt = need
        return x_copy(0, tt) if kind == "x" else dma(kind, half, tt // nstep, tt % nstep, tt % NBUF)

    def straight(u0, u1, extra=()):
        work = list(extra)
        if LOOPONLY:
            return
        for u in range(u0, u1):
            for need in needs(u):
                copy_of(need).wait()
                if need[0] == "x":
                    work.append((prep_x(0, 0, need[2], 0, SQ), SQ // 16, u - u0, 0.9))
                if need == (WO, 0, 0):
                    work.append(((prep_wo(0, r) for r in range(7)), 7, u - u0, 0.9))
            work += unit(u // NC, u % NC, u - u0)
        interleave(work)

    U0 = S if S > LP else S + NC
    copy_of((WQ, 0, 0)).start()
    x_copy(0, 0).start()
    for u in range(-LAGQ, U0):
        for need in needs(u):
            copy_of(need).start()
    copy_of((WQ, 0, 0)).wait()
    for r in range(7):
        prep_wq(0, r)
    for u in range(U0, U0 + NC):
        for need in needs(u):
            copy_of(need).start()
    x_copy(0, 0).wait()
    interleave([(prep_x(0, 0, 0, 0, SQ), SQ // 16, 0, 1)])
    cuts = [-LAGQ] + [c - LAGQ for c in CUTS if c - LAGQ < U0] + [U0]
    for k, (u0, u1) in enumerate(zip(cuts, cuts[1:])):
        if k == 1:
            for u in range(U0 + NC, U0 + PRE * NC):
                for need in needs(u):
                    copy_of(need).start()
        straight(u0, u1)

    def body(t, _):
        @pl.when(t == nstep + npc)
        def _():
            out_a.start()

        todo = [need for u in range(NC + S, NC + S + NC) for need in needs(u)]
        for br in range(2):
            for d in sorted({tt for _, _, tt in todo}):
                i = t + d + PRE - 1

                @pl.when(jnp.logical_and(i >= br * nstep, i < (br + 1) * nstep))
                def _():
                    for kind, half, tt in todo:
                        if tt == d:
                            dma(kind, half, br, i - br * nstep, i & (NBUF - 1)).start()

        @pl.when(t == U0 // NC)
        def _():
            x_all.start()

        def waits():
            for kind, half, tt in todo:
                dma(kind, half, 0, 0, (t + tt - 1) & (NBUF - 1)).wait()
        if EXTRA:
            pl.when(t < T - ahead)(waits)
        else:
            waits()

        @pl.when(t == x_end - npc)
        def _():
            x_all.wait()

        work = [bg_x(t), bg_out(t)]
        for u in range(S, S + NC):
            work += unit(t + u // NC, u % NC, u - S)
        interleave(work)
        return None
    n_iter = T - ahead
    jax.lax.fori_loop(U0 // NC, n_iter + EXTRA, body, None)

    u_end = S + n_iter * NC
    last = T * NC + LP + 1
    for u in range(u_end + PRE * NC, last):
        for need in needs(u):
            copy_of(need).start()
    cuts = [u_end] + [u_end + c for c in ECUTS] + [last + 1]
    fin = 0
    for u0, u1 in zip(cuts, cuts[1:]):
        extra = []
        sent = fin
        for u in range(u0, u1):
            c = u - LP - 1 - (T - 1) * NC
            extra += [(finalize(1, 1, cc, 0, RO), RO // 16, u - u0, 0.8) for cc in range(fin, c)]
            fin = max(fin, c)
        straight(u0, u1, extra)
        for cc in range(sent, fin):
            out_copy(1, cc).start()
    out_a.wait()
    for c in range(NC):
        out_copy(1, c).wait()


@jax.jit
def pallas_concat_heads__mha_block_cached__mha_block_cached__near_ridge_kernel(
        A_x, A_k_cache, A_v_cache, A_wq, A_wo, B_x, B_k_cache, B_v_cache, B_wq, B_wo):
    any_spec = pl.BlockSpec(memory_space=pl.ANY)
    nxs, nos = 28 + 3 * len(Q2), 28 + 3 * len(O2)
    out = pl.pallas_call(
        _kernel,
        in_specs=[any_spec] * 10,
        out_specs=any_spec,
        out_shape=jax.ShapeDtypeStruct((M, 2 * D), BF16),
        scratch_shapes=[
            pltpu.VMEM((2, M, D), BF16),
            pltpu.VMEM((3 + EXTRA // 8, nxs, M // 4, 128), BF16),
            pltpu.VMEM((NBUF, B, G, SK, DH), BF16),
            pltpu.VMEM((NBUF, B, G, SK, DH), BF16),
            pltpu.VMEM((NBUF, D, G * DH), BF16),
            pltpu.VMEM((NBUF, G * DH, D), BF16),
            pltpu.VMEM((nxs, 128, 128), BF16),
            pltpu.VMEM((nos, 128, 128), BF16),
            pltpu.VMEM((2, G, M, DH), BF16),
            pltpu.VMEM((G, M, DH if PAD else SK), BF16),
            pltpu.VMEM((G, M, DH), F32),
            pltpu.VMEM((nos, M // 4, DH), BF16),
            pltpu.VMEM((2 + EXTRA // 8, 7, M // 2, D // 2), F32),
            pltpu.VMEM((3, M, D), BF16),
            pltpu.SemaphoreType.DMA((2, NC)),
            pltpu.SemaphoreType.DMA((4, 2, NBUF)),
            pltpu.SemaphoreType.DMA((2, NC)),
        ],
        compiler_params=pltpu.CompilerParams(vmem_limit_bytes=110 * 1024 * 1024, disable_bounds_checks=True, flags=FLAGS),
    )(A_x.reshape(M, D), A_k_cache, A_v_cache, A_wq, A_wo,
      B_x.reshape(M, D), B_k_cache, B_v_cache, B_wq, B_wo)
    return out.reshape(B, SQ, 2 * D)
```

```python
import jax
import jax.numpy as jnp
import numpy as np
import jax.experimental.pallas as pl
import jax.experimental.pallas.tpu as pltpu

B, SQ, D, H, SK, DH = 16, 80, 512, 32, 80, 128
M = B * SQ
G = 4
NC = 4
CB = B // NC
CR = CB * SQ
R = CR // 2
NSTEP = H // G
T = 2 * NSTEP
NBUF = 4
AHEAD = 2
SPLIT = (1, 2, 3, 4)
BASE = [sum(7 if k in SPLIT else 4 for k in range(r)) for r in range(8)]
LAG = dict(q=3, k=0, p=-1, o=-2)
PLACE = [dict(q=(0.0, 0.7), k=(0.0, 0.7), p=(0.0, 0.95), o=(0.25, 0.673)),
         dict(q=(0.0, 0.7), k=(0.0, 0.7), p=(0.0, 0.95), o=(0.308, 0.692)),
         dict(q=(0.0, 0.7), k=(0.0, 0.7), p=(0.0, 0.95), o=(0.308, 0.692)),
         dict(q=(0.0, 0.7), k=(0.0, 0.7), p=(0.018, 0.95), o=(0.314, 0.676))]
PLACE_X = (2.193, 1.683)
TERM_SHARE = 0.692
DRAIN_CUTS = (2, 5, 6)
OUT_A_SPAN = 0.9
EXACT_RCP = False
START1, START2 = 0, 3
SCALE_LOG2E = float(DH ** -0.5 * np.log2(np.e))
F32, BF16, U32 = jnp.float32, jnp.bfloat16, jnp.uint32
WQ, KK, VV, WO = range(4)
QUAD = [(a, b) for a in range(2) for b in range(2)]

LHS = (((0, 0), (1, 1), 1), ((1, 0), (1, 1), 1), ((0, 0),), ((1, 1),),
       ((0, 0), (0, 1), 1), ((1, 0), (0, 0), -1), ((0, 1), (1, 1), -1))
RHS = (((0, 0), (1, 1), 1), ((0, 0),), ((0, 1), (1, 1), -1), ((1, 0), (0, 0), -1),
       ((1, 1),), ((0, 0), (0, 1), 1), ((1, 0), (1, 1), 1))


def term(spec, block):
    if len(spec) == 1:
        return block(*spec[0])
    a, b = block(*spec[0]).astype(F32), block(*spec[1]).astype(F32)
    return a + b if spec[2] > 0 else a - b


def tiles(side, r, block):
    quarter = [[term(side[r], lambda i, j: block(2 * i + a, 2 * j + b)) for b in range(2)] for a in range(2)]
    if r in SPLIT:
        return [term(spec, lambda i, j: quarter[i][j]) for spec in side]
    return [quarter[a][b] for a, b in QUAD]


def strassen(product, emit):
    m2 = yield from product(1)
    m4 = yield from product(3)
    emit(1, 0, m2 + m4)
    m1 = yield from product(0)
    c11, c22 = m1 + m4, m1 - m2
    m5 = yield from product(4)
    c11 = c11 - m5
    m3 = yield from product(2)
    emit(0, 1, m3 + m5)
    c22 = c22 + m3
    m7 = yield from product(6)
    emit(0, 0, c11 + m7)
    m6 = yield from product(5)
    emit(1, 1, c22 + m6)


def grid2(tile):
    return jnp.concatenate([jnp.concatenate([tile(i, j) for j in range(2)], 1) for i in range(2)], 0)


def block_dot(lhs, rhs, r, emit):
    if r in SPLIT:
        def product(k):
            m = jnp.dot(lhs(BASE[r] + k), rhs(BASE[r] + k), preferred_element_type=F32)
            yield
            return m
        yield from strassen(product, emit)
    else:
        m = jnp.dot(grid2(lambda i, j: lhs(BASE[r] + 2 * i + j)), grid2(lambda i, j: rhs(BASE[r] + 2 * i + j)),
                    preferred_element_type=F32)
        for _ in range(7):
            yield
        for i, j in QUAD:
            emit(i, j, m[i * SQ:(i + 1) * SQ, j * 128:(j + 1) * 128])


def drain(gen):
    for _ in gen:
        pass


def interleave(jobs):
    at = [[(i + 0.5) / n for i in range(n)] if isinstance(n, int) else n for _, n, _, _ in jobs]
    order = sorted((job[2] + job[3] * x, k) for k, job in enumerate(jobs) for x in at[k])
    left = [len(a) for a in at]
    for _, k in order:
        next(jobs[k][0])
        left[k] -= 1
        if left[k] == 0:
            drain(jobs[k][0])


def rows(start, size):
    if not isinstance(start, int):
        start = pl.multiple_of(start, 16 if size % 16 == 0 else 8)
    return pl.ds(start, size)


def load(ref, idx, batch=None):
    if batch is not None:
        idx = (*idx, rows(batch * (SQ // 2), SQ // 2))
    return pltpu.bitcast(ref.bitcast(U32)[idx], BF16)


def pad_keys(a):
    return jnp.concatenate([a, jnp.zeros((DH - SK, DH), BF16)], axis=0)


def _kernel(ax, ak, av, awq, awo, bx, bk, bv, bwq, bwo, out,
            xbuf, xs, kbuf, vbuf, wqbuf, wobuf, wqs, wos, qs, ps, os_, acc, obuf, sem_io, sem_in):
    sources = ((awq, ak, av, awo), (bwq, bk, bv, bwo))

    def dma(kind, br, g, slot):
        src, sem = sources[br][kind], sem_in.at[kind, slot]
        col = g * G * DH
        cols = pl.ds(col if isinstance(col, int) else pl.multiple_of(col, G * DH), G * DH)
        if kind == WQ:
            return pltpu.make_async_copy(src.at[:, cols], wqbuf.at[slot], sem)
        if kind == WO:
            return pltpu.make_async_copy(src.at[cols, :], wobuf.at[slot], sem)
        return pltpu.make_async_copy(src.at[:, pl.ds(g * G, G)], (kbuf, vbuf)[kind - KK].at[slot], sem)

    def first_reads(u0, u1):
        res = []
        for u in range(u0, u1):
            for kind, s in ((WQ, "q"), (KK, "k"), (VV, "p"), (WO, "o")):
                t, c = divmod(u + LAG[s] + (s in "qo"), NC)
                if c == 0 and 0 <= t < T and (t > 0 or kind != WQ):
                    res.append((kind, t))
        return res

    def copies(u0, u1):
        return [dma(kind, t // NSTEP, t % NSTEP, t % NBUF) for kind, t in first_reads(u0, u1)]

    def x_a(c):
        return pltpu.make_async_copy(ax.at[rows(c * CR, CR)], xbuf.at[0, rows(c * CR, CR)], sem_io.at[c])

    def out_b(c):
        return pltpu.make_async_copy(obuf.at[1, pl.ds(c * CR, CR)], out.at[pl.ds(c * CR, CR), pl.ds(D, D)], sem_io.at[c])

    x_b = pltpu.make_async_copy(bx, xbuf.at[1], sem_io.at[NC])
    out_a = pltpu.make_async_copy(obuf.at[0], out.at[:, pl.ds(0, D)], sem_io.at[NC])

    def prep_x(src, dst, c):
        for p in range(0, SQ, 16):
            def block(i, j):
                return xbuf[src, rows(c * CR + i * SQ + p, 16), j * 128:(j + 1) * 128]
            for r in range(7):
                for k, m in enumerate(tiles(LHS, r, block)):
                    xs[dst, BASE[r] + k, rows(c * SQ + p, 16), :] = m.astype(BF16)
            yield

    def prep_w(src, dst, t, r):
        ring = t & (NBUF - 1)
        for p in range(0, 128, 64):
            def block(i, j):
                return src[ring, i * 128 + p:i * 128 + p + 64, j * 128:(j + 1) * 128]
            for k, m in enumerate(tiles(RHS, r, block)):
                dst[BASE[r] + k, p:p + 64, :] = m.astype(BF16)

    def renew_weights(t, c):
        return isinstance(c, int) and c == NC - 1 and not (isinstance(t, int) and t + 1 >= T)

    def q_proj(t, c):
        br = t // NSTEP

        def product(r):
            m = {}
            yield from block_dot(lambda k: load(xs, (br, k), c), lambda k: load(wqs, (k,)), r,
                                 lambda i, j, v: m.update({(i, j): v}))
            if renew_weights(t, c):
                prep_w(wqbuf, wqs, t + 1, r)
            return grid2(lambda i, j: m[i, j])

        def emit(i, l, v):
            for h in range(2):
                qs[l * 2 + h, rows(c * CR + i * R, R), :] = v[:, h * DH:(h + 1) * DH].astype(BF16)
        yield from strassen(product, emit)

    def scores(t, c):
        ring = t & (NBUF - 1)
        for i in range(CB):
            for h in range(G):
                b = c * CB + i
                s = jax.lax.dot_general(load(qs, (h,), b), pad_keys(load(kbuf, (ring, b, h))),
                                        (((1,), (1,)), ((), ())), preferred_element_type=F32)
                s = jnp.where(jax.lax.broadcasted_iota(jnp.int32, s.shape, 1) < SK, s, -jnp.inf)
                e = jnp.exp2((s - jnp.max(s, axis=-1, keepdims=True)) * SCALE_LOG2E)
                inv = pl.reciprocal(jnp.sum(e, axis=-1, keepdims=True), approx=not EXACT_RCP)
                ps[h, rows(b * SQ, SQ), :] = (e * inv).astype(BF16)
                yield

    def values(t, c):
        ring = t & (NBUF - 1)
        o = {}
        for i in range(CB):
            for h in range(G):
                b = c * CB + i
                o[i, h] = jnp.dot(load(ps, (h,), b), pad_keys(load(vbuf, (ring, b, h))),
                                  preferred_element_type=F32)
                yield
        for r in range(7):
            for p in range(0, SQ, 16):
                for k, m in enumerate(tiles(LHS, r, lambda i, j: o[i, j][p:p + 16])):
                    os_[BASE[r] + k, rows(c * SQ + p, 16), :] = m.astype(BF16)
                yield

    def o_proj(t, c):
        static = isinstance(t, int)
        br, first = t // NSTEP, (t & (NSTEP - 1)) == 0
        for r in ((1, 3, 4, 2, 0, 6, 5) if static and t == T - 1 else (0, 4, 2, 3, 1, 5, 6)):
            def emit(i, j, m):
                at = (br, r, rows(c * R + i * SQ, SQ), slice(j * 128, (j + 1) * 128))
                if not (static and first):
                    m = (acc[at] if static else jnp.where(first, 0.0, acc[at])) + m
                acc[at] = m
            yield from block_dot(lambda k: load(os_, (k,), c), lambda k: load(wos, (k,)), r, emit)
            if renew_weights(t, c):
                prep_w(wobuf, wos, t + 1, r)

    def assemble(br, c):
        for p in range(0, R, 16):
            for a in range(0, D // 2, 128):
                def product(r):
                    return acc[br, r, c * R + p:c * R + p + 16, a:a + 128]
                    yield

                def emit(i, l, v):
                    r0, c0 = c * CR + i * R + p, l * D // 2 + a
                    obuf[br, r0:r0 + 16, c0:c0 + 128] = v.astype(BF16)
                drain(strassen(product, emit))
            yield

    v_steps = ([(1 - TERM_SHARE) * (i + 0.5) / 16 for i in range(16)]
               + [1 - TERM_SHARE + TERM_SHARE * (i + 0.5) / 35 for i in range(35)])
    stages = dict(q=(q_proj, 49), k=(scores, 16), p=(values, v_steps), o=(o_proj, 49))

    def slot(t, c, at, place):
        jobs = []
        for s in "qkpo":
            tt, cc = t + (c + LAG[s]) // NC, (c + LAG[s]) % NC
            if not isinstance(tt, int) or 0 <= tt < T:
                jobs.append((stages[s][0](tt, cc), stages[s][1], at + place[s][0], place[s][1]))
        return jobs

    def straight(u0, u1, jobs=()):
        for cp in copies(u0, u1):
            cp.wait()
        jobs = list(jobs)
        for u in range(u0, u1):
            if (WO, 0) in first_reads(u, u + 1):
                jobs.append(((prep_w(wobuf, wos, 0, r) for r in range(7)), 7, u - u0, 0.9))
            jobs += slot(u // NC, u % NC, u - u0, PLACE[1])
        interleave(jobs)

    dma(WQ, 0, 0, 0).start()
    for c in range(NC):
        x_a(c).start()
    for cp in copies(-LAG["q"], NC):
        cp.start()
    dma(WQ, 0, 0, 0).wait()
    for r in range(7):
        prep_w(wqbuf, wqs, 0, r)
    if START1 == 0:
        for cp in copies(NC, 2 * NC):
            cp.start()

    def first_q(c, _):
        x_a(c).wait()
        drain(prep_x(0, 0, c))
        drain(q_proj(0, c))
    jax.lax.fori_loop(0, NC - 1, first_q, None)
    x_a(NC - 1).wait()
    drain(prep_x(0, 0, NC - 1))
    for k, (u0, u1) in enumerate(((0, 1), (1, 2), (2, NC)), 1):
        if k == START1:
            for cp in copies(NC, 2 * NC):
                cp.start()
        if k == START2:
            for cp in copies(2 * NC, (1 + AHEAD) * NC):
                cp.start()
        straight(u0, u1)
    x_b.start()

    reads = first_reads(NC, 2 * NC)
    x_ready = NSTEP - 1

    def body(t, _):
        for kind, tt in reads:
            dma(kind, 0, 0, (t + tt - 1) & (NBUF - 1)).wait()
        for br in range(2):
            for d in sorted({tt for _, tt in reads}):
                i = t + d + AHEAD - 1

                @pl.when(jnp.logical_and(i >= br * NSTEP, i < (br + 1) * NSTEP))
                def _():
                    for kind, tt in reads:
                        if tt == d:
                            dma(kind, br, i - br * NSTEP, i & (NBUF - 1)).start()

        @pl.when(t == x_ready - NC)
        def _():
            x_b.wait()

        jobs = [(prep_x(jnp.where(t >= x_ready - NC, 1, 0), jnp.where(t < x_ready, 1, 2), t & (NC - 1)), SQ // 16, *PLACE_X)]
        for c in range(NC):
            jobs += slot(t, c, c, PLACE[c])
        interleave(jobs)
    jax.lax.fori_loop(1, T - 1, body, None)

    u_end = (T - 1) * NC
    cuts = [u_end] + [u_end + c for c in DRAIN_CUTS] + [T * NC + 3]
    done = 0
    for u0, u1 in zip(cuts, cuts[1:]):
        jobs, sent = [], done
        for u in range(u0, u1):
            ready = u + LAG["o"] - u_end
            jobs += [(assemble(1, c), R // 16, u - u0, 0.8) for c in range(done, ready)]
            done = max(done, ready)
        if u0 == u_end:
            jobs += [(assemble(0, c), R // 16, c * OUT_A_SPAN, OUT_A_SPAN) for c in range(NC)]
        straight(u0, u1, jobs)
        if u0 == u_end:
            out_a.start()
        for c in range(sent, done):
            out_b(c).start()
    out_a.wait()
    for c in range(NC):
        out_b(c).wait()


@jax.jit
def pallas_concat_heads__mha_block_cached__mha_block_cached__near_ridge_kernel(
        A_x, A_k_cache, A_v_cache, A_wq, A_wo, B_x, B_k_cache, B_v_cache, B_wq, B_wo):
    hbm = pl.BlockSpec(memory_space=pl.ANY)
    out = pl.pallas_call(
        _kernel,
        in_specs=[hbm] * 10,
        out_specs=hbm,
        out_shape=jax.ShapeDtypeStruct((M, 2 * D), BF16),
        scratch_shapes=[
            pltpu.VMEM((2, M, D), BF16),
            pltpu.VMEM((3, BASE[7], M // 4, 128), BF16),
            pltpu.VMEM((NBUF, B, G, SK, DH), BF16),
            pltpu.VMEM((NBUF, B, G, SK, DH), BF16),
            pltpu.VMEM((NBUF, D, G * DH), BF16),
            pltpu.VMEM((NBUF, G * DH, D), BF16),
            pltpu.VMEM((BASE[7], 128, 128), BF16),
            pltpu.VMEM((BASE[7], 128, 128), BF16),
            pltpu.VMEM((G, M, DH), BF16),
            pltpu.VMEM((G, M, DH), BF16),
            pltpu.VMEM((BASE[7], M // 4, DH), BF16),
            pltpu.VMEM((2, 7, M // 2, D // 2), F32),
            pltpu.VMEM((2, M, D), BF16),
            pltpu.SemaphoreType.DMA((NC + 1,)),
            pltpu.SemaphoreType.DMA((4, NBUF)),
        ],
        compiler_params=pltpu.CompilerParams(vmem_limit_bytes=110 * 1024 * 1024, disable_bounds_checks=True),
    )(A_x.reshape(M, D), A_k_cache, A_v_cache, A_wq, A_wo,
      B_x.reshape(M, D), B_k_cache, B_v_cache, B_wq, B_wo)
    return out.reshape(B, SQ, 2 * D)
```

```python
import jax
import jax.numpy as jnp
import numpy as np
import jax.experimental.pallas as pl
import jax.experimental.pallas.tpu as pltpu

B, SQ, D, H, SK, DH = 16, 80, 512, 32, 80, 128
M = B * SQ
G = 4
NC = 4
CB = B // NC
CR = CB * SQ
R = CR // 2
NSTEP = H // G
T = 2 * NSTEP
NBUF = 4
AHEAD = 2
SPLIT = (1, 2, 3, 4)
BASE = [sum(7 if k in SPLIT else 4 for k in range(r)) for r in range(8)]
LAG = dict(q=3, k=0, p=-1, o=-2)
PLACE = [dict(q=(0.0, 0.7), k=(0.0, 0.7), p=(0.0, 0.95), o=(0.25, 0.673)),
         dict(q=(0.0, 0.7), k=(0.0, 0.7), p=(0.0, 0.95), o=(0.308, 0.692)),
         dict(q=(0.0, 0.7), k=(0.0, 0.7), p=(0.0, 0.95), o=(0.308, 0.692)),
         dict(q=(0.0, 0.7), k=(0.0, 0.7), p=(0.018, 0.95), o=(0.314, 0.676))]
PLACE_X = (2.193, 1.683)
TERM_SHARE = 0.692
DRAIN_CUTS = (3, 5, 6)
OUT_A_SPAN = 0.7
SCALE_LOG2E = float(DH ** -0.5 * np.log2(np.e))
F32, BF16, U32 = jnp.float32, jnp.bfloat16, jnp.uint32
WQ, KK, VV, WO = range(4)
QUAD = [(a, b) for a in range(2) for b in range(2)]

LHS = (((0, 0), (1, 1), 1), ((1, 0), (1, 1), 1), ((0, 0),), ((1, 1),),
       ((0, 0), (0, 1), 1), ((1, 0), (0, 0), -1), ((0, 1), (1, 1), -1))
RHS = (((0, 0), (1, 1), 1), ((0, 0),), ((0, 1), (1, 1), -1), ((1, 0), (0, 0), -1),
       ((1, 1),), ((0, 0), (0, 1), 1), ((1, 0), (1, 1), 1))


def term(spec, block):
    if len(spec) == 1:
        return block(*spec[0])
    a, b = block(*spec[0]).astype(F32), block(*spec[1]).astype(F32)
    return a + b if spec[2] > 0 else a - b


def tiles(side, r, block):
    quarter = [[term(side[r], lambda i, j: block(2 * i + a, 2 * j + b)) for b in range(2)] for a in range(2)]
    if r in SPLIT:
        return [term(spec, lambda i, j: quarter[i][j]) for spec in side]
    return [quarter[a][b] for a, b in QUAD]


def strassen(product, emit):
    m2 = yield from product(1)
    m4 = yield from product(3)
    emit(1, 0, m2 + m4)
    m1 = yield from product(0)
    c11, c22 = m1 + m4, m1 - m2
    m5 = yield from product(4)
    c11 = c11 - m5
    m3 = yield from product(2)
    emit(0, 1, m3 + m5)
    c22 = c22 + m3
    m7 = yield from product(6)
    emit(0, 0, c11 + m7)
    m6 = yield from product(5)
    emit(1, 1, c22 + m6)


def grid2(tile):
    return jnp.concatenate([jnp.concatenate([tile(i, j) for j in range(2)], 1) for i in range(2)], 0)


def block_dot(lhs, rhs, r, emit):
    if r in SPLIT:
        def product(k):
            m = jnp.dot(lhs(BASE[r] + k), rhs(BASE[r] + k), preferred_element_type=F32)
            yield
            return m
        yield from strassen(product, emit)
    else:
        m = jnp.dot(grid2(lambda i, j: lhs(BASE[r] + 2 * i + j)), grid2(lambda i, j: rhs(BASE[r] + 2 * i + j)),
                    preferred_element_type=F32)
        for _ in range(7):
            yield
        for i, j in QUAD:
            emit(i, j, m[i * SQ:(i + 1) * SQ, j * 128:(j + 1) * 128])


def drain(gen):
    for _ in gen:
        pass


def interleave(jobs):
    at = [[(i + 0.5) / n for i in range(n)] if isinstance(n, int) else n for _, n, _, _ in jobs]
    order = sorted((job[2] + job[3] * x, k) for k, job in enumerate(jobs) for x in at[k])
    left = [len(a) for a in at]
    for _, k in order:
        next(jobs[k][0])
        left[k] -= 1
        if left[k] == 0:
            drain(jobs[k][0])


def rows(start, size):
    if not isinstance(start, int):
        start = pl.multiple_of(start, 16 if size % 16 == 0 else 8)
    return pl.ds(start, size)


def load(ref, idx, batch=None):
    if batch is not None:
        idx = (*idx, rows(batch * (SQ // 2), SQ // 2))
    return pltpu.bitcast(ref.bitcast(U32)[idx], BF16)


def pad_keys(a):
    return jnp.concatenate([a, jnp.zeros((DH - SK, DH), BF16)], axis=0)


def _kernel(ax, ak, av, awq, awo, bx, bk, bv, bwq, bwo, out,
            xbuf, xs, kbuf, vbuf, wqbuf, wobuf, wqs, wos, qs, ps, os_, acc, obuf, sem_io, sem_in):
    sources = ((awq, ak, av, awo), (bwq, bk, bv, bwo))

    def dma(kind, br, g, slot):
        src, sem = sources[br][kind], sem_in.at[kind, slot]
        col = g * G * DH
        cols = pl.ds(col if isinstance(col, int) else pl.multiple_of(col, G * DH), G * DH)
        if kind == WQ:
            return pltpu.make_async_copy(src.at[:, cols], wqbuf.at[slot], sem)
        if kind == WO:
            return pltpu.make_async_copy(src.at[cols, :], wobuf.at[slot], sem)
        return pltpu.make_async_copy(src.at[:, pl.ds(g * G, G)], (kbuf, vbuf)[kind - KK].at[slot], sem)

    def first_reads(u0, u1):
        res = []
        for u in range(u0, u1):
            for kind, s in ((WQ, "q"), (KK, "k"), (VV, "p"), (WO, "o")):
                t, c = divmod(u + LAG[s] + (s in "qo"), NC)
                if c == 0 and 0 <= t < T and (t > 0 or kind != WQ):
                    res.append((kind, t))
        return res

    def copies(u0, u1):
        return [dma(kind, t // NSTEP, t % NSTEP, t % NBUF) for kind, t in first_reads(u0, u1)]

    def x_a(c):
        return pltpu.make_async_copy(ax.at[rows(c * CR, CR)], xbuf.at[0, rows(c * CR, CR)], sem_io.at[c])

    def out_b(c):
        return pltpu.make_async_copy(obuf.at[1, pl.ds(c * CR, CR)], out.at[pl.ds(c * CR, CR), pl.ds(D, D)], sem_io.at[c])

    x_b = pltpu.make_async_copy(bx, xbuf.at[1], sem_io.at[NC])
    out_a = pltpu.make_async_copy(obuf.at[0], out.at[:, pl.ds(0, D)], sem_io.at[NC])

    def prep_x(src, dst, c):
        for p in range(0, SQ, 16):
            def block(i, j):
                return xbuf[src, rows(c * CR + i * SQ + p, 16), j * 128:(j + 1) * 128]
            for r in range(7):
                for k, m in enumerate(tiles(LHS, r, block)):
                    xs[dst, BASE[r] + k, rows(c * SQ + p, 16), :] = m.astype(BF16)
            yield

    def prep_w(src, dst, t, r):
        ring = t & (NBUF - 1)
        for p in range(0, 128, 64):
            def block(i, j):
                return src[ring, i * 128 + p:i * 128 + p + 64, j * 128:(j + 1) * 128]
            for k, m in enumerate(tiles(RHS, r, block)):
                dst[BASE[r] + k, p:p + 64, :] = m.astype(BF16)

    def renew_weights(t, c):
        return isinstance(c, int) and c == NC - 1 and not (isinstance(t, int) and t + 1 >= T)

    def q_proj(t, c):
        br = t // NSTEP

        def product(r):
            m = {}
            yield from block_dot(lambda k: load(xs, (br, k), c), lambda k: load(wqs, (k,)), r,
                                 lambda i, j, v: m.update({(i, j): v}))
            if renew_weights(t, c):
                prep_w(wqbuf, wqs, t + 1, r)
            return grid2(lambda i, j: m[i, j])

        def emit(i, l, v):
            for h in range(2):
                qs[l * 2 + h, rows(c * CR + i * R, R), :] = v[:, h * DH:(h + 1) * DH].astype(BF16)
        yield from strassen(product, emit)

    def scores(t, c):
        ring = t & (NBUF - 1)
        for i in range(CB):
            for h in range(G):
                b = c * CB + i
                s = jax.lax.dot_general(load(qs, (h,), b), pad_keys(load(kbuf, (ring, b, h))),
                                        (((1,), (1,)), ((), ())), preferred_element_type=F32)
                s = jnp.where(jax.lax.broadcasted_iota(jnp.int32, s.shape, 1) < SK, s, -jnp.inf)
                e = jnp.exp2((s - jnp.max(s, axis=-1, keepdims=True)) * SCALE_LOG2E)
                inv = pl.reciprocal(jnp.sum(e, axis=-1, keepdims=True), approx=True)
                ps[h, rows(b * SQ, SQ), :] = (e * inv).astype(BF16)
                yield

    def values(t, c):
        ring = t & (NBUF - 1)
        o = {}
        for i in range(CB):
            for h in range(G):
                b = c * CB + i
                o[i, h] = jnp.dot(load(ps, (h,), b), pad_keys(load(vbuf, (ring, b, h))),
                                  preferred_element_type=F32)
                yield
        for r in range(7):
            for p in range(0, SQ, 16):
                for k, m in enumerate(tiles(LHS, r, lambda i, j: o[i, j][p:p + 16])):
                    os_[BASE[r] + k, rows(c * SQ + p, 16), :] = m.astype(BF16)
                yield

    def o_proj(t, c):
        static = isinstance(t, int)
        br, first = t // NSTEP, (t & (NSTEP - 1)) == 0
        for r in ((1, 3, 4, 2, 0, 6, 5) if static and t == T - 1 else (0, 4, 2, 3, 1, 5, 6)):
            def emit(i, j, m):
                at = (br, r, rows(c * R + i * SQ, SQ), slice(j * 128, (j + 1) * 128))
                if not (static and first):
                    m = (acc[at] if static else jnp.where(first, 0.0, acc[at])) + m
                acc[at] = m
            yield from block_dot(lambda k: load(os_, (k,), c), lambda k: load(wos, (k,)), r, emit)
            if renew_weights(t, c):
                prep_w(wobuf, wos, t + 1, r)

    def assemble(br, c):
        for p in range(0, R, 16):
            for a in range(0, D // 2, 128):
                def product(r):
                    return acc[br, r, c * R + p:c * R + p + 16, a:a + 128]
                    yield

                def emit(i, l, v):
                    r0, c0 = c * CR + i * R + p, l * D // 2 + a
                    obuf[br, r0:r0 + 16, c0:c0 + 128] = v.astype(BF16)
                drain(strassen(product, emit))
            yield

    v_steps = ([(1 - TERM_SHARE) * (i + 0.5) / 16 for i in range(16)]
               + [1 - TERM_SHARE + TERM_SHARE * (i + 0.5) / 35 for i in range(35)])
    stages = dict(q=(q_proj, 49), k=(scores, 16), p=(values, v_steps), o=(o_proj, 49))

    def slot(t, c, at, place):
        jobs = []
        for s in "qkpo":
            tt, cc = t + (c + LAG[s]) // NC, (c + LAG[s]) % NC
            if not isinstance(tt, int) or 0 <= tt < T:
                jobs.append((stages[s][0](tt, cc), stages[s][1], at + place[s][0], place[s][1]))
        return jobs

    def straight(u0, u1, jobs=()):
        for cp in copies(u0, u1):
            cp.wait()
        jobs = list(jobs)
        for u in range(u0, u1):
            if (WO, 0) in first_reads(u, u + 1):
                jobs.append(((prep_w(wobuf, wos, 0, r) for r in range(7)), 7, u - u0, 0.9))
            jobs += slot(u // NC, u % NC, u - u0, PLACE[1])
        interleave(jobs)

    dma(WQ, 0, 0, 0).start()
    for c in range(NC):
        x_a(c).start()
    for cp in copies(-LAG["q"], NC):
        cp.start()
    dma(WQ, 0, 0, 0).wait()
    for r in range(7):
        prep_w(wqbuf, wqs, 0, r)
    for cp in copies(NC, 2 * NC):
        cp.start()

    def first_q(c, _):
        x_a(c).wait()
        drain(prep_x(0, 0, c))
        drain(q_proj(0, c))
    jax.lax.fori_loop(0, NC - 1, first_q, None)
    x_a(NC - 1).wait()
    drain(prep_x(0, 0, NC - 1))
    straight(0, 1)
    straight(1, 2)
    for cp in copies(2 * NC, (1 + AHEAD) * NC):
        cp.start()
    straight(2, NC)
    x_b.start()

    reads = first_reads(NC, 2 * NC)
    x_ready = NSTEP - 1

    def body(t, _):
        for kind, tt in reads:
            dma(kind, 0, 0, (t + tt - 1) & (NBUF - 1)).wait()
        for br in range(2):
            for d in sorted({tt for _, tt in reads}):
                i = t + d + AHEAD - 1

                @pl.when(jnp.logical_and(i >= br * NSTEP, i < (br + 1) * NSTEP))
                def _():
                    for kind, tt in reads:
                        if tt == d:
                            dma(kind, br, i - br * NSTEP, i & (NBUF - 1)).start()

        @pl.when(t == x_ready - NC)
        def _():
            x_b.wait()

        jobs = [(prep_x(jnp.where(t >= x_ready - NC, 1, 0), jnp.where(t < x_ready, 1, 2), t & (NC - 1)), SQ // 16, *PLACE_X)]
        for c in range(NC):
            jobs += slot(t, c, c, PLACE[c])
        interleave(jobs)
    jax.lax.fori_loop(1, T - 1, body, None)

    u_end = (T - 1) * NC
    cuts = [u_end] + [u_end + c for c in DRAIN_CUTS] + [T * NC + 3]
    done = 0
    for u0, u1 in zip(cuts, cuts[1:]):
        jobs, sent = [], done
        for u in range(u0, u1):
            ready = u + LAG["o"] - u_end
            jobs += [(assemble(1, c), R // 16, u - u0, 0.8) for c in range(done, ready)]
            done = max(done, ready)
        if u0 == u_end:
            jobs += [(assemble(0, c), R // 16, c * OUT_A_SPAN, OUT_A_SPAN) for c in range(NC)]
        straight(u0, u1, jobs)
        if u0 == u_end:
            out_a.start()
        for c in range(sent, done):
            out_b(c).start()
    out_a.wait()
    for c in range(NC):
        out_b(c).wait()


@jax.jit
def pallas_concat_heads__mha_block_cached__mha_block_cached__near_ridge_kernel(
        A_x, A_k_cache, A_v_cache, A_wq, A_wo, B_x, B_k_cache, B_v_cache, B_wq, B_wo):
    hbm = pl.BlockSpec(memory_space=pl.ANY)
    out = pl.pallas_call(
        _kernel,
        in_specs=[hbm] * 10,
        out_specs=hbm,
        out_shape=jax.ShapeDtypeStruct((M, 2 * D), BF16),
        scratch_shapes=[
            pltpu.VMEM((2, M, D), BF16),
            pltpu.VMEM((3, BASE[7], M // 4, 128), BF16),
            pltpu.VMEM((NBUF, B, G, SK, DH), BF16),
            pltpu.VMEM((NBUF, B, G, SK, DH), BF16),
            pltpu.VMEM((NBUF, D, G * DH), BF16),
            pltpu.VMEM((NBUF, G * DH, D), BF16),
            pltpu.VMEM((BASE[7], 128, 128), BF16),
            pltpu.VMEM((BASE[7], 128, 128), BF16),
            pltpu.VMEM((G, M, DH), BF16),
            pltpu.VMEM((G, M, DH), BF16),
            pltpu.VMEM((BASE[7], M // 4, DH), BF16),
            pltpu.VMEM((2, 7, M // 2, D // 2), F32),
            pltpu.VMEM((2, M, D), BF16),
            pltpu.SemaphoreType.DMA((NC + 1,)),
            pltpu.SemaphoreType.DMA((4, NBUF)),
        ],
        compiler_params=pltpu.CompilerParams(vmem_limit_bytes=110 * 1024 * 1024, disable_bounds_checks=True),
    )(A_x.reshape(M, D), A_k_cache, A_v_cache, A_wq, A_wo,
      B_x.reshape(M, D), B_k_cache, B_v_cache, B_wq, B_wo)
    return out.reshape(B, SQ, 2 * D)
```
